```python
import os as _os
_os.environ.setdefault("JAX_PLATFORMS", "cpu")
import jax
import jax.numpy as jnp

def _softmax(x, axis=-1):
    return jax.nn.softmax(x, axis=axis)
def _gelu(x):
    return jax.nn.gelu(x, approximate=True)
def _silu(x):
    return jax.nn.silu(x)
def _sigmoid(x):
    return jax.nn.sigmoid(x)
def _layernorm(x, axis=-1, eps=1e-5):
    m = jnp.mean(x, axis=axis, keepdims=True)
    v = jnp.var(x, axis=axis, keepdims=True)
    return (x - m) / jnp.sqrt(v + eps)
def _scatter_add(tgt, idx, src, axis=0):
    return tgt.at[idx].add(src)
def _segment_sum(src, seg, n):
    return jax.ops.segment_sum(src, seg, n)
class _Rng:
    def __init__(self, key):
        self._k = key
    def _next(self):
        self._k, sub = jax.random.split(self._k)
        return sub
    def normal(self, shape):
        return jax.random.normal(self._next(), shape, dtype=jnp.bfloat16)
    def randint(self, lo, hi, shape):
        return jax.random.randint(self._next(), shape, lo, hi, dtype=jnp.int32)
    def uniform(self, shape, lo=0.0, hi=1.0):
        return jax.random.uniform(self._next(), shape, jnp.bfloat16, lo, hi)
    def permutation(self, n):
        return jax.random.permutation(self._next(), n)


kernel_name = 'sequential_preLN__mha_block__mixer_token_mlp__prompt'

def setup_inputs():
    _rng = _Rng(jax.random.key(int.from_bytes(__import__("os").urandom(4), "little")))
    _w = (lambda a: (lambda t: t.astype(jnp.bfloat16) if jnp.issubdtype(t.dtype, jnp.floating) else t)(jnp.asarray(a)))
    def _A_setup():
        B, S, D, H = 1, 2048, 448, 16
        return {
            "x": _w((lambda *s: _rng.normal(s) * 0.05)(B, S, D)),
            "wqkv": _w((lambda *s: _rng.normal(s) * 0.05)(D, 3 * D)),
            "wo": _w((lambda *s: _rng.normal(s) * 0.05)(D, D)),
        }
    _A_in = _A_setup()

    def _B_setup():
        B, S, D, F = 1, 2048, 448, 1792
        return {
            "x": _w((lambda *s: _rng.normal(s) * 0.05)(B, S, D)),
            "w1": _w((lambda *s: _rng.normal(s) * 0.2)(S, F) * (S ** -0.5)),
            "b1": _w((lambda *s: _rng.normal(s) * 0.2)(F) * 0.02),
            "w2": _w((lambda *s: _rng.normal(s) * 0.2)(F, S) * (F ** -0.5)),
            "b2": _w((lambda *s: _rng.normal(s) * 0.05)(S) * 0.02),
        }
    _B_in = _B_setup()

    return {
        "A_x": _A_in["x"],
        "A_wqkv": _A_in["wqkv"],
        "A_wo": _A_in["wo"],
        "B_x": _B_in["x"],
        "B_w1": _B_in["w1"],
        "B_b1": _B_in["b1"],
        "B_w2": _B_in["w2"],
        "B_b2": _B_in["b2"],
    }

def reference(A_x, A_wqkv, A_wo, B_x, B_w1, B_b1, B_w2, B_b2):
    def _A_ref(x, wqkv, wo):
        B, S, D = x.shape
        H = 16
        Dh = D // H
        qkv = (lambda x, *d: x.transpose(*d))((x @ wqkv).reshape(B, S, 3, H, Dh), 2, 0, 3, 1, 4)
        q, k, v = qkv[0], qkv[1], qkv[2]
        scores = jnp.einsum("bhqd,bhkd->bhqk", q, k) * (Dh ** -0.5)
        p = _softmax(scores, axis=-1)
        o = jnp.einsum("bhqk,bhkd->bhqd", p, v)
        return (lambda x, *d: x.transpose(*d))(o, 0, 2, 1, 3).reshape(B, S, D) @ wo

    def _B_ref(x, w1, b1, w2, b2):
        B, S, D = x.shape
        h = _layernorm(x, axis=-1)
        u = jnp.einsum("bsd,sf->bdf", h, w1) + b1
        u = _gelu(u)
        y = jnp.einsum("bdf,fs->bds", u, w2) + b2
        return (lambda x, *d: x.transpose(*d))(y, 0, 2, 1)

    x = A_x
    h = x + _A_ref(_layernorm(x, axis=-1), A_wqkv, A_wo)
    h2 = h + _B_ref(_layernorm(h, axis=-1), B_w1, B_b1, B_w2, B_b2)
    return h2
```

```python
import jax
import jax.numpy as jnp
import numpy as np
import jax.experimental.pallas as pl
import jax.experimental.pallas.tpu as pltpu

S, D, H, DH, F = 2048, 448, 16, 28, 1792
TQ = 512
KC = 128
UA = 2
RB = 256
RP = 256
RL = 256
FB = 512
OSPLIT = (0,512,1024,1536,1792,1920,2048)
WSPLIT = (0,1344)
ORDER = (1,0,2)
LNPOS = 0
T32 = 1
E0 = 1
GP = 4
U3 = 3
EPS = 1e-5
QSCALE = float(DH ** -0.5 * np.log2(np.e))
BF, F32, U32 = jnp.bfloat16, jnp.float32, jnp.uint32


def _dot(a, b):
    return jnp.dot(a, b, preferred_element_type=F32)


def _gelu(x):
    c = float(np.sqrt(2.0 / np.pi))
    return 0.5 * x * (1.0 + jnp.tanh(c * (x + 0.044715 * (x * x * x))))


def _ln_t(xt):
    m = jnp.mean(xt, axis=0, keepdims=True)
    xc = xt - m
    v = jnp.mean(xc * xc, axis=0, keepdims=True)
    return xc * jax.lax.rsqrt(v + EPS)


def _pack(x):
    return pltpu.bitcast(x.astype(BF), U32)


def _unpack(x):
    return pltpu.bitcast(x, BF)


def _T(x):
    return pltpu.bitcast(pltpu.bitcast(x, U32).T, F32) if T32 else x.T


def _loop(n, size, body, unroll):
    def group(j, _):
        for u in range(unroll):
            i = j * unroll + u
            body(i, pl.multiple_of(i * size, size))

    if n >= 2 * unroll:
        jax.lax.fori_loop(0, n // unroll, group, None)
    done = n // unroll * unroll if n >= 2 * unroll else 0
    for i in range(done, n):
        body(i, i * size)


def _kernel(xt_hbm, wqkv_hbm, wo_hbm, w1_hbm, b1_ref, w2_hbm, b2_ref, o_hbm,
            xt_v, wqkv_v, wo_v, w1_v, w2_v, o_v, sems, wsems, xsems, osems,
            wt_s, wot_s, q_s, k_s, vt_s, ot_s, s_s, ht_s, hn2_s, g_s, b1_s, b2_s, hna, hnb):
    def x_copy(i, c0):
        return pltpu.make_async_copy(
            xt_hbm.at[:, pl.ds(c0, RB)], xt_v.at[:, pl.ds(c0, RB)], xsems.at[i])

    def o_copy(i):
        c = pl.ds(OSPLIT[i], OSPLIT[i + 1] - OSPLIT[i])
        return pltpu.make_async_copy(o_v.at[:, c], o_hbm.at[:, c], osems.at[i])

    def wq_copy(i):
        c = pl.ds(WSPLIT[i], WSPLIT[i + 1] - WSPLIT[i])
        return pltpu.make_async_copy(wqkv_hbm.at[:, c], wqkv_v.at[:, c], wsems.at[i])

    cpo = pltpu.make_async_copy(wo_hbm, wo_v, sems.at[0])
    cp1 = pltpu.make_async_copy(w1_hbm, w1_v, sems.at[1])
    cp2 = pltpu.make_async_copy(w2_hbm, w2_v, sems.at[2])
    nw, nr = len(WSPLIT) - 1, S // RB
    wq_copy(0).start()
    for r in range(E0):
        x_copy(r, r * RB).start()
    for i in range(1, nw):
        wq_copy(i).start()

    s_s[...] = jnp.zeros(s_s.shape, F32)
    b1_s[...] = b1_ref[...].astype(F32).reshape(1, F)
    b2_s[...] = b2_ref[...].astype(F32).reshape(1, S)

    def ln1(c0, dst):
        dst[...] = _pack(_ln_t(xt_v[:, pl.ds(pl.multiple_of(c0, RB), RB)].astype(F32)))

    for i in range(nw):
        wq_copy(i).wait()
        if i == nw - 1:
            for r in range(E0, 3):
                x_copy(r, r * RB).start()
        c = slice(WSPLIT[i], WSPLIT[i + 1])
        wt_s[WSPLIT[i] // 2:WSPLIT[i + 1] // 2, :] = _pack(wqkv_v[:, c].astype(F32).T)
        if i == 0:
            x_copy(0, 0).wait()
            ln1(0, hna)

    tail = jnp.where(jax.lax.broadcasted_iota(jnp.int32, (4, RB), 0) == 0, 1.0, 0.0)
    row = jax.lax.broadcasted_iota(jnp.int32, (128, RB), 0)
    z16 = jnp.zeros((16, RB), F32)
    GW = 4 * DH

    def qkv_block(c0, hn_ref, nxt_ref):
        cols = pl.ds(pl.multiple_of(c0, RB), RB)
        for g0 in range(0, 4, GP):
            for pi, part in enumerate(ORDER):
                if g0 == 0 and pi == LNPOS:
                    ln1(jnp.minimum(c0 + RB, S - RB), nxt_ref)
                r0 = part * D + g0 * GW
                y = _dot(_unpack(wt_s[r0 // 2:(r0 + GP * GW) // 2, :]), _unpack(hn_ref[...]))
                for g in range(g0, g0 + GP):
                    yg = y[(g - g0) * GW:(g - g0 + 1) * GW]
                    if part == 0:
                        q = jnp.concatenate([yg * QSCALE, z16], axis=0)
                        for j in range(4):
                            q_s[4 * g + j, :, cols] = _pack(jnp.where(
                                (row >= j * DH) & (row < (j + 1) * DH), q, 0.0))
                    elif part == 1:
                        k_s[g, pl.ds(pl.multiple_of(c0 // 2, RB // 2), RB // 2), :] = _pack(
                            _T(jnp.concatenate([yg, z16], axis=0)))
                    else:
                        for j in range(4):
                            vt_s[4 * g + j, :, cols] = _pack(jnp.concatenate(
                                [yg[j * DH:(j + 1) * DH], tail], axis=0))

    early = min(3, nr)
    for r in range(1, early):
        x_copy(r, r * RB).wait()
    for r in range(early, nr):
        x_copy(r, r * RB).start()
    cpo.start()

    def wo_block(g):
        wo = wo_v[g * GW:(g + 1) * GW, :].astype(F32)
        z4 = jnp.zeros((4, D), F32)
        wot_s[g] = _pack(jnp.concatenate(
            [p for j in range(4) for p in (wo[j * DH:(j + 1) * DH], z4)], axis=0).T)

    @pl.loop(0, nr // 2)
    def _(i):
        @pl.when(i == 1)
        def _():
            for r in range(early, nr):
                x_copy(r, r * RB).wait()

        qkv_block(2 * i * RB, hna, hnb)
        qkv_block((2 * i + 1) * RB, hnb, hna)


    def probs(c, m):
        return jnp.exp2(s_s[c * KC:(c + 1) * KC, :] - m).astype(BF)

    def contract(t, c, p):
        return _dot(_unpack(vt_s[t % H, :, c * KC:(c + 1) * KC]), p)

    def finish(t, acc):
        cols = pl.ds(pl.multiple_of((t // H) * TQ, TQ), TQ)
        ot_s[t % H, :, cols] = _pack(acc * (1.0 / acc[DH:DH + 1, :]))

    def step(ta, m, tb):
        qm = _unpack(q_s[tb % H, :, pl.ds(pl.multiple_of((tb // H) * TQ, TQ), TQ)])
        mb = acc = None
        for c in range(S // KC):
            p = probs(c, m)
            s = _dot(_unpack(k_s[tb % H // 4, c * KC // 2:(c + 1) * KC // 2, :]), qm)
            s_s[c * KC:(c + 1) * KC, :] = s
            mc = jnp.max(s.reshape(KC // 8, 8, TQ), axis=0)
            mb = mc if mb is None else jnp.maximum(mb, mc)
            o = contract(ta, c, p)
            acc = o if acc is None else acc + o
        finish(ta, acc)
        return jnp.max(mb, axis=0, keepdims=True)

    NT = H * (S // TQ)

    def body(i, m):
        pl.when(i == 1)(cp1.start)
        pl.when(i == 8)(cp2.start)
        for u in range(UA):
            t = i * UA + u
            m = step(jnp.maximum(t - 1, 0), m, t)
        return m

    m0 = jax.lax.fori_loop(0, NT // UA, body, jnp.zeros((1, TQ), F32))

    def proj_block(i, c0):
        cols = pl.ds(c0, RP)
        ot = _unpack(ot_s[:, :, cols].reshape(H * 16, RP))
        ht = xt_v[:, cols].astype(F32) + _dot(_unpack(wot_s[...]), ot)
        ht_s[:, cols] = ht
        hn2_s[:, cols] = _pack(_ln_t(ht))

    def proj_block(c0, c1):
        cols = slice(c0, c1)
        ot = _unpack(ot_s[:, :, cols].reshape(H * 16, c1 - c0))
        wot = _unpack(jnp.concatenate([wot_s[g] for g in range(4)], axis=1))
        ht = xt_v[:, cols].astype(F32) + _dot(wot, ot)
        ht_s[:, cols] = ht
        hn2_s[:, cols] = _pack(_ln_t(ht))

    cpo.wait()
    for g in range(4):
        wo_block(g)
    early_cols = list(range(0, S - TQ + 1, RP))
    n_early, n_chunk = len(early_cols) - 1, S // KC
    acc = None
    for i in range(n_early):
        for c in range(i * n_chunk // n_early, (i + 1) * n_chunk // n_early):
            o = contract(NT - 1, c, probs(c, m0))
            acc = o if acc is None else acc + o
        proj_block(early_cols[i], early_cols[i + 1])
    finish(NT - 1, acc)
    for c0 in range(S - TQ, S, RL):
        proj_block(c0, c0 + RL)

    cp1.wait()
    cp2.wait()

    def mlp1_block(i, c0, size=FB):
        cols = pl.ds(c0, size)
        u = _dot(_unpack(hn2_s[...]), w1_v[:, cols]) + b1_s[:, cols]
        g_s[:, cols] = _pack(_gelu(u))

    _loop(F // FB, FB, mlp1_block, U3)
    if F % FB:
        mlp1_block(F // FB, F // FB * FB, F % FB)

    for i in range(len(OSPLIT) - 1):
        cols = slice(OSPLIT[i], OSPLIT[i + 1])
        y = _dot(_unpack(g_s[...]), w2_v[:, cols]) + b2_s[:, cols]
        o_v[:, cols] = (y + ht_s[:, cols]).astype(o_v.dtype)
        o_copy(i).start()
    for i in range(len(OSPLIT) - 1):
        o_copy(i).wait()


@jax.jit
def pallas_sequential_preLN__mha_block__mixer_token_mlp__prompt_kernel(
    A_x: jax.Array,
    A_wqkv: jax.Array,
    A_wo: jax.Array,
    B_x: jax.Array,
    B_w1: jax.Array,
    B_b1: jax.Array,
    B_w2: jax.Array,
    B_b2: jax.Array,
):
    vmem = pl.BlockSpec(memory_space=pltpu.VMEM)
    hbm = pl.BlockSpec(memory_space=pltpu.HBM)
    out = pl.pallas_call(
        _kernel,
        out_shape=jax.ShapeDtypeStruct((D, S), A_x.dtype),
        in_specs=[hbm, hbm, hbm, hbm, vmem, hbm, vmem],
        out_specs=hbm,
        scratch_shapes=[
            pltpu.VMEM((D, S), BF),
            pltpu.VMEM((D, 3 * D), BF),
            pltpu.VMEM((D, D), BF),
            pltpu.VMEM((S, F), BF),
            pltpu.VMEM((F, S), BF),
            pltpu.VMEM((D, S), BF),
            pltpu.SemaphoreType.DMA((3,)),
            pltpu.SemaphoreType.DMA((len(WSPLIT) - 1,)),
            pltpu.SemaphoreType.DMA((S // RB,)),
            pltpu.SemaphoreType.DMA((len(OSPLIT) - 1,)),
            pltpu.VMEM((3 * D // 2, D), U32),
            pltpu.VMEM((4, D // 2, 128), U32),
            pltpu.VMEM((H, 64, S), U32),
            pltpu.VMEM((4, S // 2, 128), U32),
            pltpu.VMEM((H, 16, S), U32),
            pltpu.VMEM((H, 16, S), U32),
            pltpu.VMEM((S, TQ), F32),
            pltpu.VMEM((D, S), F32),
            pltpu.VMEM((D // 2, S), U32),
            pltpu.VMEM((D // 2, F), U32),
            pltpu.VMEM((1, F), F32),
            pltpu.VMEM((1, S), F32),
            pltpu.VMEM((D // 2, RB), U32),
            pltpu.VMEM((D // 2, RB), U32),
        ],
        compiler_params=pltpu.CompilerParams(vmem_limit_bytes=100 * 1024 * 1024),
    )(A_x.reshape(S, D).T, A_wqkv, A_wo, B_w1, B_b1, B_w2, B_b2)
    return out.T.reshape(1, S, D)
```

```python
import jax
import jax.numpy as jnp
import numpy as np
import jax.experimental.pallas as pl
import jax.experimental.pallas.tpu as pltpu

S, D, H, DH, F = 2048, 448, 16, 28, 1792
TQ = 512
KC = 128
UA = 2
RB = 256
MB = 256
EPS = 1e-5
QSCALE = float(DH ** -0.5 * np.log2(np.e))
BF, F32, U32 = jnp.bfloat16, jnp.float32, jnp.uint32


def _dot(a, b):
    return jnp.dot(a, b, preferred_element_type=F32)


def _gelu(x):
    c = float(np.sqrt(2.0 / np.pi))
    return 0.5 * x * (1.0 + jnp.tanh(c * (x + 0.044715 * (x * x * x))))


def _ln_t(xt):
    xc = xt - jnp.mean(xt, axis=0, keepdims=True)
    v = jnp.mean(xc * xc, axis=0, keepdims=True)
    return xc * jax.lax.rsqrt(v + EPS)


def _pack(x):
    return pltpu.bitcast(x.astype(BF), U32)


def _unpack(x):
    return pltpu.bitcast(x, BF)


def _operands(a):
    n = a.shape[0] // 2
    a11, a12, a21, a22 = a[:n, :128], a[:n, 128:], a[n:, :128], a[n:, 128:]
    return a11 + a22, a21 + a22, a11, a22, a11 + a12, a21 - a11, a12 - a22


def _store_lhs(a_ref, c, a):
    cols = slice(c * 128, (c + 1) * 128)
    for i, v in enumerate(_operands(a)):
        a_ref[i, :, cols] = _pack(v)


def _strassen(a_ref, b_ref, c0, k0=0, k1=None):
    k1 = b_ref.shape[0] if k1 is None else k1

    def quad(i, j):
        cols = slice(c0 + 128 * j, c0 + 128 * j + 128)
        return jnp.concatenate(
            [b_ref[r + 128 * i:r + 128 * i + 128, cols]
             for r in range(k0, k1, 256)], axis=0)

    def prod(i, b):
        return _dot(_unpack(a_ref[i, :, k0 // 2:k1 // 2]), b.astype(BF))

    b11, b22 = quad(0, 0), quad(1, 1)
    m2 = prod(1, b11)
    m5 = prod(4, b22)
    b12, b21 = quad(0, 1).astype(F32), quad(1, 0).astype(F32)
    b11, b22 = b11.astype(F32), b22.astype(F32)
    m1 = prod(0, b11 + b22)
    c22 = m1 - m2
    c11 = m1 - m5
    m3 = prod(2, b12 - b22)
    c12 = m3 + m5
    c22 = c22 + m3
    m4 = prod(3, b21 - b11)
    c21 = m2 + m4
    c11 = c11 + m4
    c22 = c22 + prod(5, b11 + b12)
    c11 = c11 + prod(6, b21 + b22)
    return jnp.concatenate([jnp.concatenate([c11, c12], axis=1),
                            jnp.concatenate([c21, c22], axis=1)], axis=0)


def _kernel(xt_hbm, wqkv_hbm, wo_hbm, w1_hbm, b1_ref, w2_hbm, b2_ref, o_hbm,
            xt_v, wqkv_v, wo_v, w1_v, w2_v, o_v, sems, xsems, osems,
            wt_s, wot_s, q_s, k_s, vt_s, ot_s, s_s, ht_s, a1_s, a2_s, b1_s, b2_s, hna, hnb):
    def x_copy(i):
        c = pl.ds(i * RB, RB)
        return pltpu.make_async_copy(xt_hbm.at[:, c], xt_v.at[:, c], xsems.at[i])

    def o_copy(i):
        c = pl.ds(i * MB, MB)
        return pltpu.make_async_copy(o_v.at[:, c], o_hbm.at[:, c], osems.at[i])

    cpq = pltpu.make_async_copy(wqkv_hbm, wqkv_v, sems.at[0])
    cpo = pltpu.make_async_copy(wo_hbm, wo_v, sems.at[1])
    cp1 = pltpu.make_async_copy(w1_hbm, w1_v, sems.at[2])
    cp2 = pltpu.make_async_copy(w2_hbm, w2_v, sems.at[3])
    cpq.start()
    x_copy(0).start()

    s_s[...] = jnp.zeros(s_s.shape, F32)
    b1_s[...] = b1_ref[...].astype(F32).reshape(1, F)
    b2_s[...] = b2_ref[...].astype(F32).reshape(1, S)

    def ln1(c0, dst):
        dst[...] = _pack(_ln_t(xt_v[:, pl.ds(pl.multiple_of(c0, RB), RB)].astype(F32)))

    nr, early = S // RB, 3
    cpq.wait()
    for r in range(1, early):
        x_copy(r).start()
    wt_s[...] = _pack(wqkv_v[...].astype(F32).T)
    x_copy(0).wait()
    ln1(0, hna)

    tail = jnp.where(jax.lax.broadcasted_iota(jnp.int32, (4, RB), 0) == 0, 1.0, 0.0)
    z4 = jnp.zeros((4, RB), F32)
    z16 = jnp.zeros((16, RB), F32)
    GW = 4 * DH

    def qkv_block(c0, hn_ref, nxt_ref):
        cols = pl.ds(pl.multiple_of(c0, RB), RB)
        rows = pl.ds(pl.multiple_of(c0 // 2, RB // 2), RB // 2)
        ln1(jnp.minimum(c0 + RB, S - RB), nxt_ref)

        def proj(part):
            w = _unpack(wt_s[part * D // 2:(part + 1) * D // 2, :])
            return _dot(w, _unpack(hn_ref[...]))

        k = proj(1)
        for g in range(4):
            kg = _pack(jnp.concatenate([k[g * GW:(g + 1) * GW], z16], axis=0).T)
            k_s[4 * g, rows, :] = kg
            for j in range(1, 4):
                k_s[4 * g + j, rows, :] = pltpu.roll(kg, 128 - j * DH, 1)
        q = proj(0) * QSCALE
        v = proj(2)
        for h in range(H):
            q_s[h, :, cols] = _pack(jnp.concatenate([q[h * DH:(h + 1) * DH], z4], axis=0))
        for h in range(H):
            vt_s[h, :, cols] = _pack(jnp.concatenate([v[h * DH:(h + 1) * DH], tail], axis=0))

    for r in range(1, early):
        x_copy(r).wait()
    for r in range(early, nr):
        x_copy(r).start()
    cpo.start()

    def wo_block(g):
        wo = wo_v[g * GW:(g + 1) * GW, :].astype(F32)
        zw = jnp.zeros((4, D), F32)
        wot_s[g] = _pack(jnp.concatenate(
            [p for j in range(4) for p in (wo[j * DH:(j + 1) * DH], zw)], axis=0).T)

    @pl.loop(0, nr // 2)
    def _(i):
        @pl.when(i == 1)
        def _():
            for r in range(early, nr):
                x_copy(r).wait()

        qkv_block(2 * i * RB, hna, hnb)
        qkv_block((2 * i + 1) * RB, hnb, hna)

    cpo.wait()


    def head(t):
        return t & (H - 1)

    def queries(t):
        return pl.ds(pl.multiple_of((t >> 4) * TQ, TQ), TQ)

    def probs(c, m):
        return jnp.exp2(s_s[c * KC:(c + 1) * KC, :] - m).astype(BF)

    def contract(t, c, p):
        return _dot(_unpack(vt_s[head(t), :, c * KC:(c + 1) * KC]), p)

    def finish(t, acc):
        ot_s[head(t), :, queries(t)] = _pack(acc * (1.0 / acc[DH:DH + 1, :]))

    def step(ta, m, tb):
        qm = _unpack(q_s[head(tb), :, queries(tb)])
        m = jnp.max(m, axis=0, keepdims=True)
        mb = acc = None
        for c in range(S // KC):
            k = _unpack(k_s[head(tb), c * KC // 2:(c + 1) * KC // 2, :])
            s = _dot(k[:, :32], qm)
            p = probs(c, m)
            s_s[c * KC:(c + 1) * KC, :] = s
            mc = jnp.max(s.reshape(KC // 8, 8, TQ), axis=0)
            mb = mc if mb is None else jnp.maximum(mb, mc)
            o = contract(ta, c, p)
            acc = o if acc is None else acc + o
        return mb, acc

    NT = H * (S // TQ)

    def body(i, carry):
        @pl.when(i == 1)
        def _():
            cp1.start()
            cp2.start()

        m, acc = carry
        for u in range(UA):
            t = i * UA + u
            finish(jnp.maximum(t - 2, 0), acc)
            m, acc = step(jnp.maximum(t - 1, 0), m, t)
        return m, acc

    m0, acc = jax.lax.fori_loop(
        0, NT // UA, body, (jnp.zeros((8, TQ), F32), jnp.ones((32, TQ), F32)))
    finish(NT - 2, acc)
    cp1.wait()
    cp2.wait()
    m0 = jnp.max(m0, axis=0, keepdims=True)

    def proj_block(c):
        wot = _unpack(jnp.concatenate([wot_s[g] for g in range(4)], axis=1))
        cols = slice(c * MB, (c + 1) * MB)
        ot = _unpack(ot_s[:, :, cols].reshape(H * 16, MB))
        ht = xt_v[:, cols].astype(F32) + _dot(wot, ot)
        ht_s[:, cols] = ht
        _store_lhs(a1_s, c, _ln_t(ht))

    n_chunk, n_early = S // KC, (S - TQ) // MB
    acc = None
    for i in range(n_early):
        for c in range(i * n_chunk // n_early, (i + 1) * n_chunk // n_early):
            o = contract(NT - 1, c, probs(c, m0))
            acc = o if acc is None else acc + o
        if i == 0:
            for g in range(4):
                wo_block(g)
        proj_block(i)
    finish(NT - 1, acc)
    for c in range(n_early, S // MB):
        if c == S // MB - 1:
            u0 = _strassen(a1_s, w1_v, 0, 0, c * MB)
        proj_block(c)


    for i in range(F // MB):
        if i == 0:
            u = u0 + _strassen(a1_s, w1_v, 0, S - MB, S)
        else:
            u = _strassen(a1_s, w1_v, i * MB)
        u = u + b1_s[:, i * MB:(i + 1) * MB]
        _store_lhs(a2_s, i, _gelu(u))

    for i in range(S // MB):
        cols = slice(i * MB, (i + 1) * MB)
        y = _strassen(a2_s, w2_v, i * MB) + b2_s[:, cols]
        o_v[:, cols] = (y + ht_s[:, cols]).astype(o_v.dtype)
        o_copy(i).start()
    for i in range(S // MB):
        o_copy(i).wait()


@jax.jit
def pallas_sequential_preLN__mha_block__mixer_token_mlp__prompt_kernel(
    A_x: jax.Array,
    A_wqkv: jax.Array,
    A_wo: jax.Array,
    B_x: jax.Array,
    B_w1: jax.Array,
    B_b1: jax.Array,
    B_w2: jax.Array,
    B_b2: jax.Array,
):
    vmem = pl.BlockSpec(memory_space=pltpu.VMEM)
    hbm = pl.BlockSpec(memory_space=pltpu.HBM)
    out = pl.pallas_call(
        _kernel,
        out_shape=jax.ShapeDtypeStruct((D, S), A_x.dtype),
        in_specs=[hbm, hbm, hbm, hbm, vmem, hbm, vmem],
        out_specs=hbm,
        scratch_shapes=[
            pltpu.VMEM((D, S), BF),
            pltpu.VMEM((D, 3 * D), BF),
            pltpu.VMEM((D, D), BF),
            pltpu.VMEM((S, F), BF),
            pltpu.VMEM((F, S), BF),
            pltpu.VMEM((D, S), BF),
            pltpu.SemaphoreType.DMA((4,)),
            pltpu.SemaphoreType.DMA((S // RB,)),
            pltpu.SemaphoreType.DMA((S // MB,)),
            pltpu.VMEM((3 * D // 2, D), U32),
            pltpu.VMEM((4, D // 2, 128), U32),
            pltpu.VMEM((H, 16, S), U32),
            pltpu.VMEM((H, S // 2, 128), U32),
            pltpu.VMEM((H, 16, S), U32),
            pltpu.VMEM((H, 16, S), U32),
            pltpu.VMEM((S, TQ), F32),
            pltpu.VMEM((D, S), F32),
            pltpu.VMEM((7, D // 4, S // 2), U32),
            pltpu.VMEM((7, D // 4, F // 2), U32),
            pltpu.VMEM((1, F), F32),
            pltpu.VMEM((1, S), F32),
            pltpu.VMEM((D // 2, RB), U32),
            pltpu.VMEM((D // 2, RB), U32),
        ],
        compiler_params=pltpu.CompilerParams(vmem_limit_bytes=100 * 1024 * 1024),
    )(A_x.reshape(S, D).T, A_wqkv, A_wo, B_w1, B_b1, B_w2, B_b2)
    return out.T.reshape(1, S, D)
```
